```python
import os as _os
_os.environ.setdefault("JAX_PLATFORMS", "cpu")
import jax
import jax.numpy as jnp

def _softmax(x, axis=-1):
    return jax.nn.softmax(x, axis=axis)
def _gelu(x):
    return jax.nn.gelu(x, approximate=True)
def _silu(x):
    return jax.nn.silu(x)
def _sigmoid(x):
    return jax.nn.sigmoid(x)
def _layernorm(x, axis=-1, eps=1e-5):
    m = jnp.mean(x, axis=axis, keepdims=True)
    v = jnp.var(x, axis=axis, keepdims=True)
    return (x - m) / jnp.sqrt(v + eps)
def _scatter_add(tgt, idx, src, axis=0):
    return tgt.at[idx].add(src)
def _segment_sum(src, seg, n):
    return jax.ops.segment_sum(src, seg, n)
class _Rng:
    def __init__(self, key):
        self._k = key
    def _next(self):
        self._k, sub = jax.random.split(self._k)
        return sub
    def normal(self, shape):
        return jax.random.normal(self._next(), shape, dtype=jnp.bfloat16)
    def randint(self, lo, hi, shape):
        return jax.random.randint(self._next(), shape, lo, hi, dtype=jnp.int32)
    def uniform(self, shape, lo=0.0, hi=1.0):
        return jax.random.uniform(self._next(), shape, jnp.bfloat16, lo, hi)
    def permutation(self, n):
        return jax.random.permutation(self._next(), n)


kernel_name = 'concat_heads__spectral_gfnet__sliding_block__prompt'

def setup_inputs():
    _rng = _Rng(jax.random.key(int.from_bytes(__import__("os").urandom(4), "little")))
    _w = (lambda a: (lambda t: t.astype(jnp.bfloat16) if jnp.issubdtype(t.dtype, jnp.floating) else t)(jnp.asarray(a)))
    def _A_setup():
        B, S, D = 1, 2048, 640
        Df = D // 2 + 1
        return {
            "x": _w((lambda *s: _rng.normal(s) * 0.05)(B, S, D)),
            "w_r": _w((lambda *s: _rng.normal(s) * 0.4)(S, Df) * 0.02),
            "w_i": _w((lambda *s: _rng.normal(s) * 0.4)(S, Df) * 0.02),
        }
    _A_in = _A_setup()

    def _B_setup():
        B, S, D = 1, 2048, 640
        return {
            "x": _w((lambda *s: _rng.normal(s) * 0.2)(B, S, D)),
            "wqkv": _w((lambda *s: _rng.normal(s) * 0.2)(D, 3 * D)),
            "wo": _w((lambda *s: _rng.normal(s) * 0.05)(D, D)),
        }
    _B_in = _B_setup()

    return {
        "A_x": _A_in["x"],
        "A_w_r": _A_in["w_r"],
        "A_w_i": _A_in["w_i"],
        "B_x": _B_in["x"],
        "B_wqkv": _B_in["wqkv"],
        "B_wo": _B_in["wo"],
    }

def reference(A_x, A_w_r, A_w_i, B_x, B_wqkv, B_wo):
    def _A_ref(x, w_r, w_i):
        B, S, D = x.shape
        X = (lambda x, axes=(-2,-1): jnp.fft.rfft2(x.astype(jnp.float32), axes=axes))(x, axes=(-2, -1))
        W = w_r + 1j * w_i
        X = X * W
        y = (lambda x, s, axes=(-2,-1): jnp.fft.irfft2(x, s=s, axes=axes).astype(jnp.bfloat16))(X, (S, D), axes=(-2, -1))
        return y

    def _B_ref(x, wqkv, wo):
        B, S, D = x.shape
        H = 32; Dh = D // H; W = 256
        qkv = (lambda x, *d: x.transpose(*d))((x @ wqkv).reshape(B, S, 3, H, Dh), 2, 0, 3, 1, 4)
        q, k, v = qkv[0], qkv[1], qkv[2]
        scores = jnp.einsum("bhqd,bhkd->bhqk", q, k) * (Dh ** -0.5)
        idx = jnp.arange(S)
        mask = (idx[:, None] - idx[None, :] >= 0) & (idx[:, None] - idx[None, :] < W)
        scores = jnp.where(mask[None, None], scores, -1e9)
        p = _softmax(scores, axis=-1)
        o = jnp.einsum("bhqk,bhkd->bhqd", p, v)
        return (lambda x, *d: x.transpose(*d))(o, 0, 2, 1, 3).reshape(B, S, D) @ wo

    a = _A_ref(A_x, A_w_r, A_w_i)
    b = _B_ref(B_x, B_wqkv, B_wo)
    return jnp.concatenate([a, b], axis=-1)
```

```python
import jax
import jax.numpy as jnp
import numpy as np
import jax.experimental.pallas as pl
import jax.experimental.pallas.tpu as pltpu

S = 2048
D = 640
H = 32
DH = 20
WIN = 256
NF = D // 2 + 1
NT = S // 128
RP = 328
RP16 = 336
NEG = -1e30
QSCALE = float(DH ** -0.5 * np.log2(np.e))
VLO = (0, 1, 2, 3, 5, 6)

C1, C2 = float(np.cos(0.4 * np.pi)), float(np.cos(0.8 * np.pi))
S1, S2 = float(np.sin(0.4 * np.pi)), float(np.sin(0.8 * np.pi))
_R2 = float(np.sqrt(0.5))


def _bf16(a):
    return np.asarray(a, np.float32).astype(jnp.bfloat16.dtype)


def _words(a):
    h = _bf16(a).view(np.uint16).astype(np.uint32)
    return h[..., 0::2, :] | (h[..., 1::2, :] << 16)


def _make_constants():
    two_pi = 2.0 * np.pi
    e = np.arange(128, dtype=np.int64)

    def trig(rhos):
        kd = np.concatenate([r + 10 * np.arange(32, dtype=np.int64) for r in rhos])
        ang = two_pi * ((kd[:, None] * e[None, :]) % D) / D
        return kd, np.cos(ang), np.sin(ang)

    alt = np.where(e % 2 == 0, 1.0, -1.0)
    _, c0, s0 = trig((0, 5))
    g0 = np.concatenate([c0, -s0, alt[None], np.zeros((15, 128))], 0)

    def gpair(lo, hi):
        _, cl, sl = trig(lo)
        _, ch, sh = trig(hi)
        re = np.concatenate([np.concatenate([cl, -sl], 1), np.concatenate([ch, sh], 1)], 0)
        im = np.concatenate([np.concatenate([-sl, -cl], 1), np.concatenate([-sh, ch], 1)], 0)
        return np.concatenate([re, im], 0)
    g14 = gpair((1, 6), (4, 9))
    g23 = gpair((2, 7), (3, 8))
    nrm = 1.0 / (S * D)
    kd0, c0, s0 = trig((0, 5))
    w0 = np.where(kd0 == 0, 1.0, 2.0)[:, None]
    hi0 = -w0 * s0
    hi0[0] = alt
    h0 = np.concatenate([w0 * c0, hi0], 0).T * nrm

    def hpair(lo, hi):
        _, cl, sl = trig(lo)
        _, ch, sh = trig(hi)
        p = np.concatenate([cl, ch, -sl, -sh], 0)
        q = np.concatenate([sl, -sh, cl, -ch], 0)
        return np.concatenate([p.T, q.T], 0) * (2.0 * nrm)
    h14 = hpair((1, 6), (4, 9))
    h23 = hpair((2, 7), (3, 8))
    gg = np.stack([g14, g23, h14, h23])
    gh = np.concatenate([g0, h0], 0)
    b = np.arange(128, dtype=np.int64)
    a = np.arange(16, dtype=np.int64)
    ss = 16 * b[None, :] + a[:, None]
    ph = two_pi * ((ss[:, :, None] * b[None, None, :]) % S) / S
    mr, mi = np.cos(ph), -np.sin(ph)
    mm = np.stack([mr, mr + mi, mi - mr], 1)
    return _words(gg), _words(gh), _words(mm)


_GG, _GH, _MM = _make_constants()
_SKIP = ()
_TOK = ('fwd', 'back')
_LAG = 2
_FL = (1, 3)
_IL = 2


def _dft4(x, sign):
    (ar, ai), (br, bi), (cr, ci), (dr, di) = x
    t0r, t0i = ar + cr, ai + ci
    t1r, t1i = ar - cr, ai - ci
    t2r, t2i = br + dr, bi + di
    t3r, t3i = br - dr, bi - di
    x0 = (t0r + t2r, t0i + t2i)
    x2 = (t0r - t2r, t0i - t2i)
    if sign < 0:
        x1 = (t1r + t3i, t1i - t3r)
        x3 = (t1r - t3i, t1i + t3r)
    else:
        x1 = (t1r - t3i, t1i + t3r)
        x3 = (t1r + t3i, t1i - t3r)
    return [x0, x1, x2, x3]


def _twiddle(z, m, sign):
    zr, zi = z
    m = m % 16
    if m == 0:
        return z
    if m == 2:
        if sign < 0:
            return ((zr + zi) * _R2, (zi - zr) * _R2)
        return ((zr - zi) * _R2, (zi + zr) * _R2)
    if m == 4:
        if sign < 0:
            return (zi, -zr)
        return (-zi, zr)
    if m == 6:
        if sign < 0:
            return ((zi - zr) * _R2, (zr + zi) * (-_R2))
        return ((zr + zi) * (-_R2), (zr - zi) * _R2)
    c = float(np.cos(2 * np.pi * m / 16))
    s = float(sign * np.sin(2 * np.pi * m / 16))
    return (zr * c - zi * s, zr * s + zi * c)


def _dft16(x, sign):
    t = []
    for a0 in range(4):
        t.append(_dft4([x[4 * a1 + a0] for a1 in range(4)], sign))
    out = [None] * 16
    for k0 in range(4):
        col = [_twiddle(t[a0][k0], a0 * k0, sign) for a0 in range(4)]
        res = _dft4(col, sign)
        for kh in range(4):
            out[k0 + 4 * kh] = res[kh]
    return out


def _dft5_real(x):
    x0, x1, x2, x3, x4 = x
    s14, d14 = x1 + x4, x1 - x4
    s23, d23 = x2 + x3, x2 - x3
    y0 = x0 + s14 + s23
    a1 = x0 + C1 * s14 + C2 * s23
    a2 = x0 + C2 * s14 + C1 * s23
    b1 = S1 * d14 + S2 * d23
    b2 = S2 * d14 - S1 * d23
    return y0, a1, b1, a2, b2


def _idft5_real(g0, p1, q1, p2, q2):
    ea = g0 + C1 * p1 + C2 * p2
    eb = g0 + C2 * p1 + C1 * p2
    oa = S1 * q1 + S2 * q2
    ob = S2 * q1 - S1 * q2
    return [g0 + p1 + p2, ea - oa, eb - ob, eb + ob, ea + oa]


def _kernel(xa_hbm, wr_hbm, wi_hbm, xb_hbm, wqkv_hbm, wo_hbm,
            gg_hbm, gh_hbm, mm_hbm, z_ref,
            out_hbm,
            xa_v, xb_v, wk_v, wq_v, wv_v, wo_v, wr_v, wi_v, wl_v, gg_v, gh_v, mm_v,
            ys, ts, kp, khat, qt, vt, wqvt, outa, outb,
            sem_in, sem_xa, sem_xb, sem_w, sem_oa, sem_ob):
    f32, bf16, u32 = jnp.float32, jnp.bfloat16, jnp.uint32
    nt_dims = (((1,), (1,)), ((), ()))

    def dot(a, b):
        return jnp.dot(a, b, preferred_element_type=f32)

    def dot_nt(a, b):
        return jax.lax.dot_general(a, b, nt_dims, preferred_element_type=f32)

    def bc(v):
        return pltpu.bitcast(v, bf16)

    def cp_in(src, dst, i):
        return pltpu.make_async_copy(src, dst, sem_in.at[i])

    c_wk = cp_in(wqkv_hbm.at[:, pl.ds(D, D)], wk_v.bitcast(bf16), 0)

    def xb_copy(i):
        return pltpu.make_async_copy(xb_hbm.at[0, pl.ds(512 * i, 512), :],
                                     xb_v.bitcast(bf16).at[pl.ds(512 * i, 512), :], sem_xb.at[i])
    c_xa = [pltpu.make_async_copy(xa_hbm.at[0, :, pl.ds(128 * c, 128)],
                                  xa_v.at[c].bitcast(bf16), sem_xa.at[c]) for c in range(5)]
    c_gg = cp_in(gg_hbm, gg_v, 1)
    c_gh = cp_in(gh_hbm, gh_v, 2)
    c_mm = cp_in(mm_hbm, mm_v, 3)
    c_wq = cp_in(wqkv_hbm.at[:, pl.ds(0, D)], wq_v, 4)
    c_wv = cp_in(wqkv_hbm.at[:, pl.ds(2 * D, D)], wv_v, 5)
    c_w = []
    for n, (src, dst) in enumerate(((wr_hbm, wr_v), (wi_hbm, wi_v))):
        for k1 in range(16):
            c_w.append(pltpu.make_async_copy(src.at[pl.ds(0, NF - 1), pl.ds(128 * k1, 128)],
                                             dst.at[k1].bitcast(bf16), sem_w.at[16 * n + k1]))
    c_wl = [cp_in(wr_hbm.at[pl.ds(NF - 1, 1), :], wl_v.at[0], 6),
            cp_in(wi_hbm.at[pl.ds(NF - 1, 1), :], wl_v.at[1], 7)]
    c_wo = cp_in(wo_hbm, wo_v.bitcast(bf16), 8)
    stages = [[xb_copy(2), xb_copy(3)], c_xa, [c_gg, c_gh, c_mm], [c_wq, c_wv]]
    for c in (c_wk, xb_copy(0), xb_copy(1)):
        c.start()

    lane = jax.lax.broadcasted_iota(jnp.int32, (8, 128), 1)
    sub8 = jax.lax.broadcasted_iota(jnp.int32, (8, 128), 0)
    zeros8 = jnp.zeros((8, 128), f32)
    zero_u = jnp.zeros((8, 128), u32)
    neg_bits = int(np.asarray(NEG, np.float32).astype(jnp.bfloat16.dtype).view(np.uint16))
    padrow = jnp.where(lane == 127, jnp.uint32(neg_bits * 0x10001), jnp.uint32(0))
    for t in range(6):
        for r in range(WIN // 16):
            kp[t, pl.ds(8 * r, 8), :] = padrow
    vt[:, pl.ds(0, WIN)] = jnp.zeros((16 * H, WIN), u32)

    c_wk.wait()
    lane128 = jax.lax.broadcasted_iota(jnp.int32, (128, 128), 1)

    def k_tile(t):
        w0 = pl.multiple_of(t * 64, 64)
        kb = dot(bc(xb_v[pl.ds(w0, 64), :]), bc(wk_v[...]))
        tiles = [kb[:, 128 * j:128 * (j + 1)] for j in range(5)]
        for tt in range(6):
            off = (120 * tt) % 128
            a = (120 * tt) // 128
            if off == 0:
                v = tiles[a]
            elif a + 1 < 5:
                sh = 128 - off
                v = jnp.where(lane128 < sh, pltpu.roll(tiles[a], sh, 1),
                              pltpu.roll(tiles[a + 1], sh, 1))
            else:
                v = pltpu.roll(tiles[a], 128 - off, 1)
            v = jnp.where(lane128 == 127, 0.0, v)
            kp[tt, pl.ds(WIN // 2 + w0, 64), :] = pltpu.bitcast(v.astype(bf16), u32)

    def k_body(i, carry):
        for n, cs in enumerate(stages):
            @pl.when(i == n)
            def _(cs=cs):
                for c in cs:
                    c.start()
        xb_copy(i).wait()
        for u in range(4):
            k_tile(4 * i + u)
        return carry
    if 'k' not in _SKIP:
        jax.lax.fori_loop(0, 4, k_body, 0)
    else:
        for cs in stages:
            for c in cs:
                c.start()
        for i in range(4):
            xb_copy(i).wait()

    for c in c_xa + [c_gg, c_gh, c_mm]:
        c.wait()
    for c in c_w + c_wl + [c_wo]:
        c.start()
    himask = jnp.uint32(0xFFFF0000)
    lo60 = lane < 60

    def khat_tile(t):
        w0 = 64 * t
        for u in range(11):
            tt = u // 2
            for r in range(4):
                av = kp[tt, pl.ds(w0 + 8 * r, 8), :]
                bv = kp[tt, pl.ds(w0 + 160 + 8 * r, 8), :]
                if u % 2 == 0:
                    keep_a = jnp.logical_or(lo60, lane == 127)
                    bs = pltpu.roll(bv, 60, 1)
                else:
                    keep_a = jnp.logical_not(lo60)
                    bs = pltpu.roll(bv, 68, 1)
                khat[t, u, pl.ds(8 * r, 8), :] = jnp.where(keep_a, av, bs)

    fw = [dict() for _ in range(16)]

    def fwd_0(a):
        j, p = a // 2, a % 2
        xe, xo = [], []
        for c in range(5):
            e = xa_v[c, pl.ds(j, 64, stride=16), :]
            o = xa_v[c, pl.ds(8 + j, 64, stride=16), :]
            xe.append(pltpu.bitcast((e << 16) if p == 0 else (e & himask), f32))
            xo.append(pltpu.bitcast((o << 16) if p == 0 else (o & himask), f32))
        ye, yo = _dft5_real(xe), _dft5_real(xo)
        fw[a]['y'] = [pltpu.pack_elementwise([ye[i], yo[i]], packed_dtype=bf16) for i in range(5)]

    def fwd_1(a):
        y = fw[a].pop('y')
        z0 = dot_nt(bc(gh_v[pl.ds(0, 72), :]), bc(y[0]))
        z14 = dot_nt(bc(gg_v[0]), bc(jnp.concatenate([y[1], y[2]], axis=1)))
        z23 = dot_nt(bc(gg_v[1]), bc(jnp.concatenate([y[3], y[4]], axis=1)))
        zr = jnp.concatenate(
            [z0[0:32], z14[0:32], z23[0:32], z23[64:96], z14[64:96],
             z0[32:64], z14[32:64], z23[32:64], z23[96:128], z14[96:128], z0[128:144]], 0)
        zi = jnp.concatenate(
            [z0[64:96], z14[128:160], z23[128:160], z23[192:224], z14[192:224],
             z0[96:128], z14[160:192], z23[160:192], z23[224:256], z14[224:256],
             zeros8, zeros8], 0)
        fw[a]['z'] = [(zr + zi).astype(bf16), zi.astype(bf16), zr.astype(bf16)]

    def fwd_2(a):
        z = fw[a].pop('z')
        k1 = dot(z[0], bc(mm_v[a, 0]))
        k2 = dot(z[1], bc(mm_v[a, 1]))
        k3 = dot(z[2], bc(mm_v[a, 2]))
        ys[a, :, pl.ds(0, 128)] = (k1 - k2)[:RP]
        ys[a, :, pl.ds(128, 128)] = (k1 + k3)[:RP]

    if 'fwd' not in _SKIP:
        for step in range(16 + _FL[1]):
            if step < 16:
                fwd_0(step)
                khat_tile(step)
            if 0 <= step - _FL[0] < 16:
                fwd_1(step - _FL[0])
            if 0 <= step - _FL[1] < 16:
                fwd_2(step - _FL[1])

    c_wq.wait()
    c_wv.wait()
    for j in range(5):
        wqvt[pl.ds(0, D // 2), pl.ds(128 * j, 128)] = pltpu.bitcast(wq_v[pl.ds(128 * j, 128), :].T, u32)
        wqvt[pl.ds(D // 2, D // 2), pl.ds(128 * j, 128)] = pltpu.bitcast(
            wv_v[pl.ds(128 * j, 128), :].T, u32)

    for c in c_w + c_wl:
        c.wait()
    hi64 = lane >= 64

    never = lane + z_ref[0] < 0

    def qv_tile(t, tok=None):
        x = xb_v[pl.ds(64 * t, 64), :]
        if tok is not None:
            x0 = jnp.where(never, pltpu.bitcast(tok, u32), x[0:8, 0:128])
            x = jnp.concatenate([jnp.concatenate([x0, x[8:, 0:128]], 0), x[:, 128:]], 1)
        qv = dot_nt(bc(wqvt[...]), bc(x))
        q = qv[:D + 48] * QSCALE
        for h in range(H):
            tt, i = h // 6, h % 6
            j = (i + 3) % 6
            base = 120 * tt
            pa, pb = [], []
            for g in range(4):
                row = 16 * VLO[i] + 8 * g
                lo, hi = 20 * i - row, 20 * i + 20 - row
                if hi <= 0 or lo >= 8:
                    va = zeros8
                else:
                    va = q[base + row:base + row + 8]
                    if lo > 0:
                        va = jnp.where(sub8 >= lo, va, 0.0)
                    if hi < 8:
                        va = jnp.where(sub8 < hi, va, 0.0)
                if row == 120:
                    va = jnp.where(sub8 == 7, 1.0, va)
                pa.append(va)
                row = 16 * VLO[j] + 8 * g
                lo, hi = 20 * j - row, 20 * j + 20 - row
                if hi <= 0 or lo >= 8:
                    vb = zeros8
                else:
                    src = base + row + 20 * i - 20 * j
                    if src < 0:
                        vb = jnp.concatenate([zeros8[:-src], q[0:8 + src]], 0)
                    else:
                        vb = q[src:src + 8]
                    keep = hi64
                    if lo > 0:
                        keep = jnp.logical_and(keep, sub8 >= lo)
                    if hi < 8:
                        keep = jnp.logical_and(keep, sub8 < hi)
                    vb = jnp.where(keep, vb, 0.0)
                if row == 120:
                    vb = jnp.where(jnp.logical_and(sub8 == 7, lane < 64), 1.0, vb)
                pb.append(vb)
            qt[t, h] = pltpu.bitcast(jnp.concatenate(pa + pb, 0).astype(bf16), u32)
        for j in range(H // 2):
            g = [qv[D + 40 * j + 8 * i:D + 40 * j + 8 * i + 8] for i in range(5)]
            ev = jnp.concatenate(
                [g[0], g[1], jnp.where(sub8 < 4, g[2], jnp.where(sub8 == 4, 1.0, 0.0)), zeros8], 0)
            od = jnp.concatenate(
                [jnp.where(sub8 >= 4, g[2], jnp.where(sub8 == 0, 1.0, 0.0)), g[3], g[4], zeros8], 0)
            vt[pl.ds(32 * j, 32), pl.ds(WIN + 128 * t, 128)] = pltpu.bitcast(
                jnp.concatenate([ev, od], 0).astype(bf16), u32)
        return qv[0:8]

    def spectrum(r0, wr, wi, tok=None):
        x = [(ys[a, pl.ds(r0, 8), pl.ds(0, 128)], ys[a, pl.ds(r0, 8), pl.ds(128, 128)])
             for a in range(16)]
        if tok is not None:
            x[0] = (jnp.where(never, tok, x[0][0]), x[0][1])
        xf = _dft16(x, -1)
        xw = []
        for k1 in range(16):
            xr, xi = xf[k1]
            ar, ai = wr[k1], wi[k1]
            xw.append((xr * ar - xi * ai, xr * ai + xi * ar))
        return _dft16(xw, +1)

    def put_t(r0, halves):
        for a in range(16):
            tr = jnp.concatenate([halves[0][a][0], halves[1][a][0]], 0)
            ti = jnp.concatenate([halves[0][a][1], halves[1][a][1]], 0)
            for c, v in enumerate((tr + ti, tr, ti)):
                ts[a, c, pl.ds(r0 // 2, 8), :] = pltpu.bitcast(v.astype(bf16), u32)

    def mid_block(i, tok=None):
        if i < 20:
            rho, m0 = i // 2, 16 * (i % 2)
            halves = []
            for hh in range(2):
                st = rho // 2 + 5 * (m0 + 8 * hh)
                ws = []
                for ref in (wr_v, wi_v):
                    w = [ref[k1, pl.ds(st, 8, stride=5), :] for k1 in range(16)]
                    w = [pltpu.bitcast((v << 16) if rho % 2 == 0 else (v & himask), f32) for v in w]
                    ws.append(w)
                halves.append(spectrum(16 * i + 8 * hh, ws[0], ws[1], tok))
            put_t(16 * i, halves)
            return halves[1][15][1]
        else:
            wr = [jnp.broadcast_to(wl_v[0, :, pl.ds(128 * k1, 128)].astype(f32), (8, 128))
                  for k1 in range(16)]
            wi = [jnp.broadcast_to(wl_v[1, :, pl.ds(128 * k1, 128)].astype(f32), (8, 128))
                  for k1 in range(16)]
            last = spectrum(320, wr, wi, tok)
            put_t(320, [last, [(zeros8, zeros8)] * 16])
            return last[15][1]

    if 'qv' not in _SKIP:
        nblk = 21
        done = 0
        mtok = {}
        for t in range(NT):
            tok = qv_tile(t, mtok.get(t - _LAG) if 'back' in _TOK else None)
            upto = ((t + 1) * nblk + NT - 1) // NT
            if 'mid' not in _SKIP:
                for i in range(done, upto):
                    mtok[t] = mid_block(i, tok if 'fwd' in _TOK else None)
            done = upto

    iv = [dict() for _ in range(16)]

    def inv_1(a):
        k1 = dot_nt(bc(ts[a, 0]), bc(mm_v[a, 0]))
        k2 = dot_nt(bc(ts[a, 1]), bc(mm_v[a, 1]))
        k3 = dot_nt(bc(ts[a, 2]), bc(mm_v[a, 2]))
        ur, ui = k1 + k3, k1 - k2

        def rows(v, rhos):
            return [v[32 * r:32 * r + 32] for r in rhos]
        ui0 = jnp.concatenate(
            [jnp.where(sub8 == 0, ur[320:328], ui[0:8]), ui[8:32]], 0)
        iv[a]['st'] = [
            jnp.concatenate(rows(ur, (0, 5)) + [ui0] + rows(ui, (5,)), 0).astype(bf16),
            jnp.concatenate(rows(ur, (1, 6, 4, 9)) + rows(ui, (1, 6, 4, 9)), 0).astype(bf16),
            jnp.concatenate(rows(ur, (2, 7, 3, 8)) + rows(ui, (2, 7, 3, 8)), 0).astype(bf16)]

    def inv_2(a):
        st0, st14, st23 = iv[a].pop('st')
        g0 = dot(bc(gh_v[pl.ds(72, 64), :]), st0)
        pq1 = dot(bc(gg_v[2]), st14)
        pq2 = dot(bc(gg_v[3]), st23)
        iv[a]['y'] = _idft5_real(g0, pq1[:128], pq1[128:], pq2[:128], pq2[128:])
        if a % 2 == 1:
            y0, y1 = iv[a - 1].pop('y'), iv[a].pop('y')
            for c in range(5):
                words = pltpu.pack_elementwise([y0[c], y1[c]], packed_dtype=bf16)
                outa[c, pl.ds(a // 2, 128, stride=8), :] = words.T

    if 'inv' not in _SKIP:
        for step in range(16 + _IL):
            if step < 16:
                inv_1(step)
            if 0 <= step - _IL < 16:
                inv_2(step - _IL)
    c_outa = [pltpu.make_async_copy(outa.at[c].bitcast(bf16), out_hbm.at[0, :, pl.ds(128 * c, 128)],
                                    sem_oa.at[c]) for c in range(5)]
    for c in c_outa:
        c.start()

    c_wo.wait()
    r128 = jax.lax.broadcasted_iota(jnp.int32, (128, 128), 0)
    upper = r128 > lane128
    lomask = jnp.where(jax.lax.broadcasted_iota(jnp.int32, (16, 128), 1) < 64,
                       jnp.uint32(0xFFFFFFFF), jnp.uint32(0))
    last_all = jnp.where(sub8 == 7, jnp.uint32(0x3F800000), jnp.uint32(0))
    last_lo = jnp.where(jnp.logical_and(sub8 == 7, lane < 64), jnp.uint32(0x3F800000), jnp.uint32(0))
    TQ = 2

    def outb_copy(i):
        rows = 128 * TQ
        return pltpu.make_async_copy(outb.at[pl.ds(rows * i, rows), :],
                                     out_hbm.at[0, pl.ds(rows * i, rows), pl.ds(D, D)],
                                     sem_ob.at[i])

    def attn_body(tb, carry):
        n = H * TQ
        st = [dict() for _ in range(n)]

        def tq(k):
            return tb * TQ + k // H

        def stage_a(k):
            h = k % H
            i, j = h % 6, (h % 6 + 3) % 6
            t = tq(k)
            w0 = pl.multiple_of(t * 64, 64)
            qa = qt[t, h, pl.ds(0, 16), :]
            qb = qt[t, h, pl.ds(16, 16), :]
            pa, pb = [zero_u] * 8, [zero_u] * 8
            pa[VLO[i]], pa[VLO[i] + 1] = qa[:8], qa[8:]
            ql = qa & lomask
            pb[VLO[i]], pb[VLO[i] + 1] = ql[:8], ql[8:]
            pb[VLO[j]], pb[VLO[j] + 1] = qb[:8], qb[8:]
            if i != 5:
                pa[7] = last_all
                if j != 5:
                    pb[7] = last_lo
            qw, qw2 = bc(jnp.concatenate(pa, 0)), bc(jnp.concatenate(pb, 0))
            xa = dot(bc(kp[h // 6, pl.ds(w0 + 32, 64), :]), qw)
            xb = dot(bc(kp[h // 6, pl.ds(w0 + 96, 64), :]), qw)
            hh = dot(bc(khat[t, h // 3]), qw2)
            sa = jnp.concatenate([jnp.where(upper[:64], hh, xb[64:]),
                                  jnp.where(upper[64:], xa[:64], hh)], 0)
            sb = jnp.concatenate([xa[64:], xb[:64]], 0)
            st[k].update(sa=sa, sb=sb, m=jnp.max(jnp.maximum(sa, sb), axis=0, keepdims=True))

        def stage_e(k):
            s = st[k]
            m = s.pop('m')
            pa = jnp.exp2(s.pop('sa') - m)
            s['p0'] = jnp.where(upper, pa, 0.0).astype(bf16)
            s['p2'] = jnp.where(upper, 0.0, pa).astype(bf16)
            s['p1'] = jnp.exp2(s.pop('sb') - m).astype(bf16)

        def stage_v(k):
            h = k % H
            r0 = pl.multiple_of(tq(k) * 128, 128)
            s = st[k]
            r = None
            for c, name in ((0, 'p0'), (2, 'p2'), (1, 'p1')):
                d = dot(bc(vt[pl.ds(16 * h, 16), pl.ds(r0 + 128 * c, 128)]), s.pop(name))
                r = d if r is None else r + d
            s['r'] = r
            if h == H - 1:
                groups = []
                for kk in range(k - H + 1, k + 1, 2):
                    ra, rb = st[kk].pop('r'), st[kk + 1].pop('r')
                    ia = 1.0 / ra[20:21]
                    ib = 1.0 / rb[0:1]
                    groups += [ra[0:8] * ia, ra[8:16] * ia,
                               jnp.where(sub8 < 4, ra[16:24] * ia, rb[0:8] * ib),
                               rb[8:16] * ib, rb[16:24] * ib]
                o = jnp.concatenate(groups, axis=0).astype(bf16).T
                outb[pl.ds(r0, 128), :] = dot(o, bc(wo_v[...])).astype(bf16)

        for step in range(n + 3):
            if step < n:
                stage_a(step)
            if 0 <= step - 2 < n:
                stage_e(step - 2)
            if 0 <= step - 3 < n:
                stage_v(step - 3)
        outb_copy(tb).start()
        return carry
    if 'attn' not in _SKIP:
        jax.lax.fori_loop(0, NT // TQ, attn_body, 0)

    for c in c_outa:
        c.wait()
    if 'attn' not in _SKIP:
        for i in range(NT // TQ):
            outb_copy(i).wait()


def _call(xa, wr, wi, xb, wqkv, wo, interpret=False):
    bf16, f32, u32 = jnp.bfloat16, jnp.float32, jnp.uint32
    V = pltpu.VMEM
    scratch = [
        V((5, S // 2, 128), u32),
        V((S // 2, D), u32),
        V((D // 2, D), u32),
        V((D, D), bf16), V((D, D), bf16),
        V((D // 2, D), u32),
        V((16, 160, 128), u32), V((16, 160, 128), u32),
        V((2, 1, S), bf16),
        V((4, 128, 256), u32),
        V((136, 128), u32),
        V((16, 3, 64, 128), u32),
        V((16, RP, 256), f32),
        V((16, 3, RP16 // 2, 128), u32),
        V((6, (S + WIN) // 2, 128), u32),
        V((NT, 11, 32, 128), u32),
        V((NT, H, 32, 128), u32),
        V((16 * H, S + WIN), u32),
        V((D, D), u32),
        V((5, S // 2, 128), u32),
        V((S, D), bf16),
        pltpu.SemaphoreType.DMA((9,)),
        pltpu.SemaphoreType.DMA((5,)),
        pltpu.SemaphoreType.DMA((4,)),
        pltpu.SemaphoreType.DMA((32,)),
        pltpu.SemaphoreType.DMA((5,)),
        pltpu.SemaphoreType.DMA((NT // 2,)),
    ]
    any_spec = pl.BlockSpec(memory_space=pl.ANY)
    return pl.pallas_call(
        lambda *refs: _kernel(*refs),
        out_shape=jax.ShapeDtypeStruct((1, S, 2 * D), bf16),
        in_specs=[any_spec] * 9 + [pl.BlockSpec(memory_space=pltpu.SMEM)],
        out_specs=any_spec,
        scratch_shapes=scratch,
        compiler_params=pltpu.CompilerParams(vmem_limit_bytes=100 * 1024 * 1024),
        interpret=interpret,
    )(xa, wr.T, wi.T, xb, wqkv, wo, _GG, _GH, _MM, np.zeros((1,), np.int32))


@jax.jit
def pallas_concat_heads__spectral_gfnet__sliding_block__prompt_kernel(
    A_x: jax.Array,
    A_w_r: jax.Array,
    A_w_i: jax.Array,
    B_x: jax.Array,
    B_wqkv: jax.Array,
    B_wo: jax.Array,
):
    return _call(A_x, A_w_r, A_w_i, B_x, B_wqkv, B_wo)
```

```python
import jax
import jax.numpy as jnp
import numpy as np
import jax.experimental.pallas as pl
import jax.experimental.pallas.tpu as pltpu

S = 2048
D = 640
H = 32
DH = 20
WIN = 256
NF = D // 2 + 1
NT = S // 128
RP = 328
RP16 = 336
NEG = -1e30
QSCALE = float(DH ** -0.5 * np.log2(np.e))
VLO = (0, 1, 2, 3, 5, 6)

C1, C2 = float(np.cos(0.4 * np.pi)), float(np.cos(0.8 * np.pi))
S1, S2 = float(np.sin(0.4 * np.pi)), float(np.sin(0.8 * np.pi))
_R2 = float(np.sqrt(0.5))


def _bf16(a):
    return np.asarray(a, np.float32).astype(jnp.bfloat16.dtype)


def _words(a):
    h = _bf16(a).view(np.uint16).astype(np.uint32)
    return h[..., 0::2, :] | (h[..., 1::2, :] << 16)


def _make_constants():
    two_pi = 2.0 * np.pi
    e = np.arange(128, dtype=np.int64)

    def trig(rhos):
        kd = np.concatenate([r + 10 * np.arange(32, dtype=np.int64) for r in rhos])
        ang = two_pi * ((kd[:, None] * e[None, :]) % D) / D
        return kd, np.cos(ang), np.sin(ang)

    alt = np.where(e % 2 == 0, 1.0, -1.0)
    _, c0, s0 = trig((0, 5))
    g0 = np.concatenate([c0, -s0, alt[None], np.zeros((15, 128))], 0)

    def gpair(lo, hi):
        _, cl, sl = trig(lo)
        _, ch, sh = trig(hi)
        re = np.concatenate([np.concatenate([cl, -sl], 1), np.concatenate([ch, sh], 1)], 0)
        im = np.concatenate([np.concatenate([-sl, -cl], 1), np.concatenate([-sh, ch], 1)], 0)
        return np.concatenate([re, im], 0)
    g14 = gpair((1, 6), (4, 9))
    g23 = gpair((2, 7), (3, 8))
    nrm = 1.0 / (S * D)
    kd0, c0, s0 = trig((0, 5))
    w0 = np.where(kd0 == 0, 1.0, 2.0)[:, None]
    hi0 = -w0 * s0
    hi0[0] = alt
    h0 = np.concatenate([w0 * c0, hi0], 0).T * nrm

    def hpair(lo, hi):
        _, cl, sl = trig(lo)
        _, ch, sh = trig(hi)
        p = np.concatenate([cl, ch, -sl, -sh], 0)
        q = np.concatenate([sl, -sh, cl, -ch], 0)
        return np.concatenate([p.T, q.T], 0) * (2.0 * nrm)
    h14 = hpair((1, 6), (4, 9))
    h23 = hpair((2, 7), (3, 8))
    gg = np.stack([g14, g23, h14, h23])
    gh = np.concatenate([g0, h0], 0)
    b = np.arange(128, dtype=np.int64)
    a = np.arange(16, dtype=np.int64)
    ph = two_pi * ((b[:, None] * b[None, :]) % 128) / 128
    pt = two_pi * (a[:, None] * b[None, :]) / S
    tw = np.concatenate([np.cos(ph), -np.sin(ph), np.cos(pt), -np.sin(pt)], 0)
    return _words(gg), _words(gh), tw.astype(np.float32)


_GG, _GH, _TW = _make_constants()


def _dft4(x, sign):
    (ar, ai), (br, bi), (cr, ci), (dr, di) = x
    t0r, t0i = ar + cr, ai + ci
    t1r, t1i = ar - cr, ai - ci
    t2r, t2i = br + dr, bi + di
    t3r, t3i = br - dr, bi - di
    x0 = (t0r + t2r, t0i + t2i)
    x2 = (t0r - t2r, t0i - t2i)
    if sign < 0:
        x1 = (t1r + t3i, t1i - t3r)
        x3 = (t1r - t3i, t1i + t3r)
    else:
        x1 = (t1r - t3i, t1i + t3r)
        x3 = (t1r + t3i, t1i - t3r)
    return [x0, x1, x2, x3]


def _twiddle(z, m, sign):
    zr, zi = z
    m = m % 16
    if m == 0:
        return z
    if m == 2:
        if sign < 0:
            return ((zr + zi) * _R2, (zi - zr) * _R2)
        return ((zr - zi) * _R2, (zi + zr) * _R2)
    if m == 4:
        if sign < 0:
            return (zi, -zr)
        return (-zi, zr)
    if m == 6:
        if sign < 0:
            return ((zi - zr) * _R2, (zr + zi) * (-_R2))
        return ((zr + zi) * (-_R2), (zr - zi) * _R2)
    c = float(np.cos(2 * np.pi * m / 16))
    s = float(sign * np.sin(2 * np.pi * m / 16))
    return (zr * c - zi * s, zr * s + zi * c)


def _dft16(x, sign):
    t = []
    for a0 in range(4):
        t.append(_dft4([x[4 * a1 + a0] for a1 in range(4)], sign))
    out = [None] * 16
    for k0 in range(4):
        col = [_twiddle(t[a0][k0], a0 * k0, sign) for a0 in range(4)]
        res = _dft4(col, sign)
        for kh in range(4):
            out[k0 + 4 * kh] = res[kh]
    return out


def _dft5_real(x):
    x0, x1, x2, x3, x4 = x
    s14, d14 = x1 + x4, x1 - x4
    s23, d23 = x2 + x3, x2 - x3
    y0 = x0 + s14 + s23
    a1 = x0 + C1 * s14 + C2 * s23
    a2 = x0 + C2 * s14 + C1 * s23
    b1 = S1 * d14 + S2 * d23
    b2 = S2 * d14 - S1 * d23
    return y0, a1, b1, a2, b2


def _idft5_real(g0, p1, q1, p2, q2):
    ea = g0 + C1 * p1 + C2 * p2
    eb = g0 + C2 * p1 + C1 * p2
    oa = S1 * q1 + S2 * q2
    ob = S2 * q1 - S1 * q2
    return [g0 + p1 + p2, ea - oa, eb - ob, eb + ob, ea + oa]


def _kernel(xa_hbm, wr_hbm, wi_hbm, xb_hbm, wqkv_hbm, wo_hbm,
            gg_hbm, gh_hbm, tw_hbm,
            out_hbm,
            xa_v, xb_v, wk_v, wq_v, wv_v, wo_v, wr_v, wi_v, wl_v, gg_v, gh_v, tw_v,
            ys, ts, kp, khat, qt, vt, wqvt, outa, outb, ssc,
            sem_in, sem_wk, sem_xa, sem_xb, sem_w, sem_oa, sem_ob):
    f32, bf16, u32 = jnp.float32, jnp.bfloat16, jnp.uint32
    nt_dims = (((1,), (1,)), ((), ()))

    def dot(a, b):
        return jnp.dot(a, b, preferred_element_type=f32)

    def dot_nt(a, b):
        return jax.lax.dot_general(a, b, nt_dims, preferred_element_type=f32)

    def mult(v, m):
        return v if isinstance(v, int) else pl.multiple_of(v, m)

    def bc(v):
        return pltpu.bitcast(v, bf16)

    def words(v):
        return pltpu.bitcast(v.astype(bf16), u32)

    def cp_in(src, dst, i):
        return pltpu.make_async_copy(src, dst, sem_in.at[i])

    def xb_copy(i):
        r0 = pl.multiple_of(512 * i, 128)
        return pltpu.make_async_copy(xb_hbm.at[0, pl.ds(r0, 512), :],
                                     xb_v.at[pl.ds(r0, 512), :], sem_xb.at[i])

    c_wk = [pltpu.make_async_copy(wqkv_hbm.at[pl.ds(128 * j, 128), pl.ds(D, D)],
                                  wk_v.at[pl.ds(128 * j, 128), :], sem_wk.at[j]) for j in range(5)]
    c_xa = [pltpu.make_async_copy(xa_hbm.at[0, :, pl.ds(128 * c, 128)],
                                  xa_v.at[pl.ds(S * c, S), :], sem_xa.at[c]) for c in range(5)]
    c_gg = cp_in(gg_hbm, gg_v, 0)
    c_gh = cp_in(gh_hbm, gh_v, 1)
    c_tw = cp_in(tw_hbm, tw_v, 2)
    c_wq = cp_in(wqkv_hbm.at[:, pl.ds(0, D)], wq_v, 3)
    c_wv = cp_in(wqkv_hbm.at[:, pl.ds(2 * D, D)], wv_v, 4)
    c_w = []
    for n, (src, dst) in enumerate(((wr_hbm, wr_v), (wi_hbm, wi_v))):
        for k1 in range(16):
            c_w.append(pltpu.make_async_copy(src.at[pl.ds(0, NF - 1), pl.ds(128 * k1, 128)],
                                             dst.at[pl.ds(320 * k1, 320), :],
                                             sem_w.at[16 * n + k1]))
    c_wl = [cp_in(wr_hbm.at[pl.ds(NF - 1, 1), :], wl_v.at[0], 5),
            cp_in(wi_hbm.at[pl.ds(NF - 1, 1), :], wl_v.at[1], 6)]
    c_wo = cp_in(wo_hbm, wo_v, 7)
    for c in c_wk + [xb_copy(0)]:
        c.start()
    stages = [[xb_copy(2), c_gg, c_gh, c_tw], [xb_copy(3)] + c_xa, [c_wq, c_wv], []]

    lane = jax.lax.broadcasted_iota(jnp.int32, (8, 128), 1)
    sub8 = jax.lax.broadcasted_iota(jnp.int32, (8, 128), 0)
    zeros8 = jnp.zeros((8, 128), f32)
    zero_u = jnp.zeros((8, 128), u32)

    for c in c_wk:
        c.wait()
    xb_copy(1).start()
    lane128 = jax.lax.broadcasted_iota(jnp.int32, (128, 128), 1)

    def k_tile(t):
        w0 = mult(t * 64, 64)
        kb = dot(xb_v[pl.ds(2 * w0, 128), :], wk_v[...])
        tiles = [kb[:, 128 * j:128 * (j + 1)] for j in range(5)]
        for tt in range(6):
            off = (120 * tt) % 128
            a = (120 * tt) // 128
            if off == 0:
                v = tiles[a]
            elif a + 1 < 5:
                sh = 128 - off
                v = jnp.where(lane128 < sh, pltpu.roll(tiles[a], sh, 1),
                              pltpu.roll(tiles[a + 1], sh, 1))
            else:
                v = pltpu.roll(tiles[a], 128 - off, 1)
            kp[pl.ds(w0, 64), pl.ds(128 * tt, 128)] = words(v)

    def w_transpose(src, r0, j):
        wqvt[pl.ds(r0, D // 2), pl.ds(128 * j, 128)] = pltpu.bitcast(
            src[pl.ds(128 * j, 128), :].T, u32)

    lo60 = lane < 60

    def khat_tile(t):
        w0 = 64 * t
        h0 = 32 * t
        for u in range(11):
            tt = u // 2
            for r in range(4):
                av = kp[pl.ds(w0 - 128 + 8 * r, 8), pl.ds(128 * tt, 128)]
                bv = kp[pl.ds(w0 + 32 + 8 * r, 8), pl.ds(128 * tt, 128)]
                if u % 2 == 0:
                    keep_a = lo60
                    bs = pltpu.roll(bv, 60, 1)
                else:
                    keep_a = jnp.logical_not(lo60)
                    bs = pltpu.roll(bv, 68, 1)
                khat[pl.ds(h0 + 8 * r, 8), pl.ds(128 * u, 128)] = jnp.where(keep_a, av, bs)

    def k_body(i, carry):
        for n, cs in enumerate(stages):
            @pl.when(i == n)
            def _(cs=cs):
                for c in cs:
                    c.start()
        xb_copy(i).wait()
        for u in range(4):
            k_tile(4 * i + u)
        return carry
    jax.lax.fori_loop(0, 4, k_body, 0)

    for c in c_xa + [c_gg, c_gh, c_tw]:
        c.wait()
    for c in c_w + c_wl + [c_wo]:
        c.start()
    himask = jnp.uint32(0xFFFF0000)

    def dft_mats(a):
        fr, fi = tw_v[pl.ds(0, 128), :], tw_v[pl.ds(128, 128), :]
        tr, ti = tw_v[pl.ds(256 + a, 1), :], tw_v[pl.ds(272 + a, 1), :]
        mr, mi = fr * tr - fi * ti, fr * ti + fi * tr
        return [v.astype(bf16) for v in (mr, mr + mi, mi - mr)]

    xa_w = xa_v.bitcast(u32)
    wr_w, wi_w, outa_w = wr_v.bitcast(u32), wi_v.bitcast(u32), outa.bitcast(u32)
    fw = [dict() for _ in range(16)]

    def fwd_0(a):
        j, p = a // 2, a % 2
        xe, xo = [], []
        for c in range(5):
            e = xa_w[pl.ds(1024 * c + j, 64, stride=8), :]
            o = xa_w[pl.ds(1024 * c + 512 + j, 64, stride=8), :]
            xe.append(pltpu.bitcast((e << 16) if p == 0 else (e & himask), f32))
            xo.append(pltpu.bitcast((o << 16) if p == 0 else (o & himask), f32))
        ye, yo = _dft5_real(xe), _dft5_real(xo)
        fw[a]['y'] = [jnp.concatenate([ye[i], yo[i]], 0).astype(bf16) for i in range(5)]

    def fwd_1(a):
        y = fw[a].pop('y')
        z0 = dot_nt(bc(gh_v[pl.ds(0, 72), :]), y[0])
        z14 = dot_nt(bc(gg_v[0]), jnp.concatenate([y[1], y[2]], axis=1))
        z23 = dot_nt(bc(gg_v[1]), jnp.concatenate([y[3], y[4]], axis=1))
        zr = jnp.concatenate(
            [z0[0:32], z14[0:32], z23[0:32], z23[64:96], z14[64:96],
             z0[32:64], z14[32:64], z23[32:64], z23[96:128], z14[96:128], z0[128:144]], 0)
        zi = jnp.concatenate(
            [z0[64:96], z14[128:160], z23[128:160], z23[192:224], z14[192:224],
             z0[96:128], z14[160:192], z23[160:192], z23[224:256], z14[224:256],
             jnp.zeros((16, 128), f32)], 0)
        fw[a]['z'] = [(zr + zi).astype(bf16), zi.astype(bf16), zr.astype(bf16)]

    def fwd_2(a):
        z = fw[a].pop('z')
        ms = dft_mats(a)
        k1 = dot(z[0], ms[0])
        k2 = dot(z[1], ms[1])
        k3 = dot(z[2], ms[2])
        ys[a, :, pl.ds(0, 128)] = (k1 - k2)[:RP]
        ys[a, :, pl.ds(128, 128)] = (k1 + k3)[:RP]

    row16 = jax.lax.broadcasted_iota(jnp.int32, (16, 128), 0)
    hi64_16 = jax.lax.broadcasted_iota(jnp.int32, (16, 128), 1) >= 64
    never = tw_v[pl.ds(0, 8), :] > 2.0

    def qv_tile(t, tok=None):
        x = pltpu.bitcast(xb_v[pl.ds(128 * t, 128), :], u32)
        if tok is not None:
            x0 = jnp.where(never, pltpu.bitcast(tok, u32), x[0:8, 0:128])
            x = jnp.concatenate([jnp.concatenate([x0, x[8:, 0:128]], 0), x[:, 128:]], 1)
        qv = dot_nt(bc(wqvt[pl.ds(0, D), :]), bc(x))
        q = qv[:D + 48] * QSCALE
        for h in range(H):
            tt, i = h // 6, h % 6
            j = (i + 3) % 6
            base = 120 * tt
            for part, (pos, shift) in enumerate(((i, 0), (j, 20 * i - 20 * j))):
                for g in range(2):
                    row = 16 * (VLO[pos] + g)
                    lo, hi = 20 * pos - row, 20 * pos + 20 - row
                    src = base + row + shift
                    if src < 0:
                        v = jnp.concatenate([jnp.zeros((-src, 128), f32), q[0:16 + src]], 0)
                    else:
                        v = q[src:src + 16]
                    keep = hi64_16 if part == 1 else None
                    if lo > 0:
                        keep = (row16 >= lo) if keep is None else jnp.logical_and(keep, row16 >= lo)
                    if hi < 16:
                        keep = (row16 < hi) if keep is None else jnp.logical_and(keep, row16 < hi)
                    if keep is not None:
                        v = jnp.where(keep, v, 0.0)
                    qt[pl.ds(16 * (H * t + h) + 8 * g, 8), pl.ds(128 * part, 128)] = words(v)
        for j in range(H // 2):
            r = D + 40 * j
            pieces = [qv[r:r + 16], jnp.where(row16 == 4, 1.0, qv[r + 16:r + 32]),
                      jnp.where(row16 == 0, 1.0, qv[r + 16:r + 32])]
            if j < H // 2 - 1:
                pieces.append(qv[r + 32:r + 48])
            else:
                pieces.append(jnp.concatenate([qv[r + 32:r + 40], zeros8], 0))
            for g, v in enumerate(pieces):
                vt[pl.ds(32 * j + 8 * g, 8), pl.ds(128 * t, 128)] = words(v)
        return qv[0:8]

    def spectrum(r0, wr, wi, tok=None):
        x = [(ys[a, pl.ds(r0, 8), pl.ds(0, 128)], ys[a, pl.ds(r0, 8), pl.ds(128, 128)])
             for a in range(16)]
        if tok is not None:
            x[0] = (jnp.where(never, tok, x[0][0]), x[0][1])
        xf = _dft16(x, -1)
        xw = []
        for k1 in range(16):
            xr, xi = xf[k1]
            ar, ai = wr[k1], wi[k1]
            xw.append((xr * ar - xi * ai, xr * ai + xi * ar))
        return _dft16(xw, +1)

    def put_t(w0, halves):
        for a in range(16):
            tr = jnp.concatenate([halves[0][a][0], halves[1][a][0]], 0)
            ti = jnp.concatenate([halves[0][a][1], halves[1][a][1]], 0)
            for c, v in enumerate((tr + ti, tr, ti)):
                ts[pl.ds(168 * a + w0, 8), pl.ds(128 * c, 128)] = words(v)

    def mid_block(i, tok):
        rho = i // 2
        halves = []
        for hh in range(2):
            st = rho // 2 + 80 * (i % 2) + 40 * hh
            ws = []
            for ref in (wr_w, wi_w):
                w = [ref[pl.ds(160 * k1 + st, 8, stride=5), :] for k1 in range(16)]
                ws.append([pltpu.bitcast((v << 16) if rho % 2 == 0 else (v & himask), f32)
                           for v in w])
            halves.append(spectrum(16 * i + 8 * hh, ws[0], ws[1], tok))
        put_t(8 * i, halves)
        return halves[1][15][1]

    def mid_last():
        wr = [jnp.broadcast_to(wl_v[0, :, pl.ds(128 * k1, 128)].astype(f32), (8, 128))
              for k1 in range(16)]
        wi = [jnp.broadcast_to(wl_v[1, :, pl.ds(128 * k1, 128)].astype(f32), (8, 128))
              for k1 in range(16)]
        put_t(160, [spectrum(320, wr, wi), [(zeros8, zeros8)] * 16])

    for step in range(16 + 3):
        if step == 10:
            c_wq.wait()
            c_wv.wait()
        if 10 <= step < 15:
            w_transpose(wq_v, 0, step - 10)
            w_transpose(wv_v, D // 2, step - 10)
        if step < 16:
            fwd_0(step)
        if 2 <= step < 16:
            khat_tile(step)
        if 0 <= step - 1 < 16:
            fwd_1(step - 1)
        if 0 <= step - 3 < 16:
            fwd_2(step - 3)
    for c in c_w + c_wl:
        c.wait()
    done = 0
    mtk = {}
    for t in range(NT):
        tok = qv_tile(t, mtk.get(t - 4))
        upto = ((t + 1) * 21 + NT - 1) // NT
        for i in range(done, upto):
            if i < 20:
                mtk[t] = mid_block(i, tok)
            else:
                mid_last()
        done = upto

    iv = [dict() for _ in range(16)]
    row32 = jax.lax.broadcasted_iota(jnp.int32, (32, 128), 0)

    def inv_1(a):
        ms = dft_mats(a)
        k1 = dot_nt(bc(ts[pl.ds(168 * a, 168), pl.ds(0, 128)]), ms[0])
        k2 = dot_nt(bc(ts[pl.ds(168 * a, 168), pl.ds(128, 128)]), ms[1])
        k3 = dot_nt(bc(ts[pl.ds(168 * a, 168), pl.ds(256, 128)]), ms[2])
        ur, ui = k1 + k3, k1 - k2

        def rows(v, rhos):
            return [v[32 * r:32 * r + 32] for r in rhos]
        ui0 = jnp.where(row32 == 0, jnp.broadcast_to(ur[320:321], (32, 128)), ui[0:32])
        iv[a]['st'] = [
            jnp.concatenate(rows(ur, (0, 5)) + [ui0] + rows(ui, (5,)), 0).astype(bf16),
            jnp.concatenate(rows(ur, (1, 6, 4, 9)) + rows(ui, (1, 6, 4, 9)), 0).astype(bf16),
            jnp.concatenate(rows(ur, (2, 7, 3, 8)) + rows(ui, (2, 7, 3, 8)), 0).astype(bf16)]

    def inv_2(a):
        st0, st14, st23 = iv[a].pop('st')
        g0 = dot(bc(gh_v[pl.ds(72, 64), :]), st0)
        pq1 = dot(bc(gg_v[2]), st14)
        pq2 = dot(bc(gg_v[3]), st23)
        iv[a]['y'] = _idft5_real(g0, pq1[:128], pq1[128:], pq2[:128], pq2[128:])
        if a % 2 == 1:
            y0, y1 = iv[a - 1].pop('y'), iv[a].pop('y')
            for c in range(5):
                lo = pltpu.bitcast(y0[c].astype(bf16).astype(f32), u32)
                hi = pltpu.bitcast(y1[c].astype(bf16).astype(f32), u32)
                outa_w[pl.ds(1024 * c + a // 2, 128, stride=8), :] = ((lo >> 16) | hi).T

    def inv_step(step):
        if step < 16:
            inv_1(step)
        if 0 <= step - 2 < 16:
            inv_2(step - 2)

    c_outa = [pltpu.make_async_copy(outa.at[pl.ds(S * c, S), :],
                                    out_hbm.at[0, :, pl.ds(128 * c, 128)], sem_oa.at[c])
              for c in range(5)]

    c_wo.wait()
    r128 = jax.lax.broadcasted_iota(jnp.int32, (128, 128), 0)
    upper = r128 > lane128
    lomask = jnp.where(jax.lax.broadcasted_iota(jnp.int32, (16, 128), 1) < 64,
                       jnp.uint32(0xFFFFFFFF), jnp.uint32(0))
    TQ = 2
    LA = 3

    def outb_copy(i):
        return pltpu.make_async_copy(outb.at[pl.ds(128 * i, 128), :],
                                     out_hbm.at[0, pl.ds(128 * i, 128), pl.ds(D, D)],
                                     sem_ob.at[i])

    def stage_a(t, h):
        i, j = h % 6, (h % 6 + 3) % 6
        w0 = mult(t * 64, 64)
        q0 = mult((t * H + h) * 16, 16)
        qa = qt[pl.ds(q0, 16), pl.ds(0, 128)]
        qb = qt[pl.ds(q0, 16), pl.ds(128, 128)]
        pa, pb = [zero_u] * 8, [zero_u] * 8
        pa[VLO[i]], pa[VLO[i] + 1] = qa[:8], qa[8:]
        ql = qa & lomask
        pb[VLO[i]], pb[VLO[i] + 1] = ql[:8], ql[8:]
        pb[VLO[j]], pb[VLO[j] + 1] = qb[:8], qb[8:]
        qw, qw2 = bc(jnp.concatenate(pa, 0)), bc(jnp.concatenate(pb, 0))
        ktile = pl.ds(128 * (h // 6), 128)
        if isinstance(t, int) and t < 2:
            sa = jnp.where(upper, NEG, dot(bc(kp[pl.ds(64 * t, 64), ktile]), qw))
            if t == 0:
                return dict(sa=sa, m=jnp.max(sa, axis=0, keepdims=True))
            sb = dot(bc(kp[pl.ds(0, 64), ktile]), qw)
            return dict(sa=sa, sb=sb, m=jnp.max(jnp.maximum(sa, sb), axis=0, keepdims=True))
        xa = dot(bc(kp[pl.ds(w0 - 96, 64), ktile]), qw)
        xb = dot(bc(kp[pl.ds(w0 - 32, 64), ktile]), qw)
        hh = dot(bc(khat[pl.ds(mult(t * 32, 32), 32), pl.ds(128 * (h // 3), 128)]), qw2)
        sa = jnp.concatenate([jnp.where(upper[:64], hh, xb[64:]),
                              jnp.where(upper[64:], xa[:64], hh)], 0)
        sb = jnp.concatenate([xa[64:], xb[:64]], 0)
        return dict(sa=sa, sb=sb, m=jnp.max(jnp.maximum(sa, sb), axis=0, keepdims=True))

    def park(j, s_):
        ssc[j, pl.ds(0, 128), :] = s_['sa']
        ssc[j, pl.ds(128, 128), :] = s_['sb']
        ssc[j, pl.ds(256, 8), :] = jnp.broadcast_to(s_['m'], (8, 128))

    def attn_body(tb, carry):
        n = H * TQ
        st = [dict() for _ in range(n)]
        early = isinstance(tb, int)

        def tq(k):
            return tb * TQ + k // H

        def stage_e(k):
            s_ = st[k]
            m = s_.pop('m')
            pa = jnp.exp2(s_.pop('sa') - m)
            if early:
                s_['p2'] = pa.astype(bf16)
            else:
                s_['p0'] = jnp.where(upper, pa, 0.0).astype(bf16)
                s_['p2'] = jnp.where(upper, 0.0, pa).astype(bf16)
            if 'sb' in s_:
                s_['p1'] = jnp.exp2(s_.pop('sb') - m).astype(bf16)

        def stage_v(k):
            h = k % H
            r0 = mult(tq(k) * 128, 128)
            s_ = st[k]
            r = None
            for c, name in ((0, 'p0'), (2, 'p2'), (1, 'p1')):
                if name not in s_:
                    continue
                d = dot(bc(vt[pl.ds(16 * h, 16), pl.ds(r0 - WIN + 128 * c, 128)]), s_.pop(name))
                r = d if r is None else r + d
            s_['r'] = r
            if h == H - 1:
                groups = []
                for kk in range(k - H + 1, k + 1, 2):
                    ra, rb = st[kk].pop('r'), st[kk + 1].pop('r')
                    ia = 1.0 / ra[20:21]
                    ib = 1.0 / rb[0:1]
                    groups += [ra[0:8] * ia, ra[8:16] * ia,
                               jnp.where(sub8 < 4, ra[16:24] * ia, rb[0:8] * ib),
                               rb[8:16] * ib, rb[16:24] * ib]
                o = jnp.concatenate(groups, axis=0).astype(bf16).T
                outb[pl.ds(r0, 128), :] = dot(o, wo_v[...]).astype(bf16)
                outb_copy(tq(k)).start()

        for k in range(LA):
            if early:
                st[k] = stage_a(0, k)
            else:
                st[k].update(sa=ssc[k, pl.ds(0, 128), :], sb=ssc[k, pl.ds(128, 128), :],
                             m=ssc[k, pl.ds(256, 1), :])
        for step in range(n + 1):
            if step < n:
                k = step + LA
                if k < n:
                    st[k] = stage_a(tq(k), k % H)
                else:
                    park(k - n, stage_a(TQ if early else jnp.minimum(tb * TQ + TQ, NT - 1), k - n))
                stage_e(step)
            if step >= 1:
                stage_v(step - 1)
            if early and step % 2 == 1 and step // 2 < 18:
                inv_step(step // 2)
        return carry
    attn_body(0, 0)
    for c in c_outa:
        c.start()
    jax.lax.fori_loop(1, NT // TQ, attn_body, 0)

    for c in c_outa:
        c.wait()
    for i in range(NT):
        outb_copy(i).wait()


def _call(xa, wr, wi, xb, wqkv, wo):
    bf16, f32, u32 = jnp.bfloat16, jnp.float32, jnp.uint32
    V = pltpu.VMEM
    scratch = [
        V((5 * S, 128), bf16),
        V((S, D), bf16),
        V((D, D), bf16),
        V((D, D), bf16), V((D, D), bf16),
        V((D, D), bf16),
        V((16 * 320, 128), bf16), V((16 * 320, 128), bf16),
        V((2, 1, S), bf16),
        V((4, 128, 256), u32),
        V((136, 128), u32),
        V((2 * 128 + 2 * 16, 128), f32),
        V((16, RP, 256), f32),
        V((16 * RP16 // 2, 3 * 128), u32),
        V((S // 2, 6 * 128), u32),
        V((NT * 32, 11 * 128), u32),
        V((NT * H * 16, 256), u32),
        V((16 * H, S), u32),
        V((D, D), u32),
        V((5 * S, 128), bf16),
        V((S, D), bf16),
        V((3, 264, 128), f32),
        pltpu.SemaphoreType.DMA((8,)),
        pltpu.SemaphoreType.DMA((5,)),
        pltpu.SemaphoreType.DMA((5,)),
        pltpu.SemaphoreType.DMA((4,)),
        pltpu.SemaphoreType.DMA((32,)),
        pltpu.SemaphoreType.DMA((5,)),
        pltpu.SemaphoreType.DMA((NT,)),
    ]
    any_spec = pl.BlockSpec(memory_space=pl.ANY)
    return pl.pallas_call(
        _kernel,
        out_shape=jax.ShapeDtypeStruct((1, S, 2 * D), bf16),
        in_specs=[any_spec] * 9,
        out_specs=any_spec,
        scratch_shapes=scratch,
        compiler_params=pltpu.CompilerParams(vmem_limit_bytes=100 * 1024 * 1024),
    )(xa, wr.T, wi.T, xb, wqkv, wo, _GG, _GH, _TW)


@jax.jit
def pallas_concat_heads__spectral_gfnet__sliding_block__prompt_kernel(
    A_x: jax.Array,
    A_w_r: jax.Array,
    A_w_i: jax.Array,
    B_x: jax.Array,
    B_wqkv: jax.Array,
    B_wo: jax.Array,
):
    return _call(A_x, A_w_r, A_w_i, B_x, B_wqkv, B_wo)
```

```python
import jax
import jax.numpy as jnp
import numpy as np
import jax.experimental.pallas as pl
import jax.experimental.pallas.tpu as pltpu

S = 2048
D = 640
H = 32
DH = 20
WIN = 256
NF = D // 2 + 1
NT = S // 128
RP = 328
RP16 = 336
NEG = -1e30
QSCALE = float(DH ** -0.5 * np.log2(np.e))
VLO = (0, 1, 2, 3, 5, 6)

C1, C2 = float(np.cos(0.4 * np.pi)), float(np.cos(0.8 * np.pi))
S1, S2 = float(np.sin(0.4 * np.pi)), float(np.sin(0.8 * np.pi))
_R2 = float(np.sqrt(0.5))


def _bf16(a):
    return np.asarray(a, np.float32).astype(jnp.bfloat16.dtype)


def _words(a):
    h = _bf16(a).view(np.uint16).astype(np.uint32)
    return h[..., 0::2, :] | (h[..., 1::2, :] << 16)


def _make_constants():
    two_pi = 2.0 * np.pi
    e = np.arange(128, dtype=np.int64)

    def trig(rhos):
        kd = np.concatenate([r + 10 * np.arange(32, dtype=np.int64) for r in rhos])
        ang = two_pi * ((kd[:, None] * e[None, :]) % D) / D
        return kd, np.cos(ang), np.sin(ang)

    alt = np.where(e % 2 == 0, 1.0, -1.0)
    _, c0, s0 = trig((0, 5))
    g0 = np.concatenate([c0, -s0, alt[None], np.zeros((15, 128))], 0)

    def gpair(lo, hi):
        _, cl, sl = trig(lo)
        _, ch, sh = trig(hi)
        re = np.concatenate([np.concatenate([cl, -sl], 1), np.concatenate([ch, sh], 1)], 0)
        im = np.concatenate([np.concatenate([-sl, -cl], 1), np.concatenate([-sh, ch], 1)], 0)
        return np.concatenate([re, im], 0)
    g14 = gpair((1, 6), (4, 9))
    g23 = gpair((2, 7), (3, 8))
    nrm = 1.0 / (S * D)
    kd0, c0, s0 = trig((0, 5))
    w0 = np.where(kd0 == 0, 1.0, 2.0)[:, None]
    hi0 = -w0 * s0
    hi0[0] = alt
    h0 = np.concatenate([w0 * c0, hi0], 0).T * nrm

    def hpair(lo, hi):
        _, cl, sl = trig(lo)
        _, ch, sh = trig(hi)
        p = np.concatenate([cl, ch, -sl, -sh], 0)
        q = np.concatenate([sl, -sh, cl, -ch], 0)
        return np.concatenate([p.T, q.T], 0) * (2.0 * nrm)
    h14 = hpair((1, 6), (4, 9))
    h23 = hpair((2, 7), (3, 8))
    gg = np.stack([g14, g23, h14, h23])
    gh = np.concatenate([g0, h0], 0)
    b = np.arange(128, dtype=np.int64)
    a = np.arange(16, dtype=np.int64)
    ph = two_pi * ((b[:, None] * b[None, :]) % 128) / 128
    pt = two_pi * (a[:, None] * b[None, :]) / S
    tw = np.concatenate([np.cos(ph), -np.sin(ph), np.cos(pt), -np.sin(pt)], 0)
    return _words(gg), _words(gh), tw.astype(np.float32)


_GG, _GH, _TW = _make_constants()


def _dft4(x, sign):
    (ar, ai), (br, bi), (cr, ci), (dr, di) = x
    t0r, t0i = ar + cr, ai + ci
    t1r, t1i = ar - cr, ai - ci
    t2r, t2i = br + dr, bi + di
    t3r, t3i = br - dr, bi - di
    x0 = (t0r + t2r, t0i + t2i)
    x2 = (t0r - t2r, t0i - t2i)
    if sign < 0:
        x1 = (t1r + t3i, t1i - t3r)
        x3 = (t1r - t3i, t1i + t3r)
    else:
        x1 = (t1r - t3i, t1i + t3r)
        x3 = (t1r + t3i, t1i - t3r)
    return [x0, x1, x2, x3]


def _twiddle(z, m, sign):
    zr, zi = z
    m = m % 16
    if m == 0:
        return z
    if m == 2:
        if sign < 0:
            return ((zr + zi) * _R2, (zi - zr) * _R2)
        return ((zr - zi) * _R2, (zi + zr) * _R2)
    if m == 4:
        if sign < 0:
            return (zi, -zr)
        return (-zi, zr)
    if m == 6:
        if sign < 0:
            return ((zi - zr) * _R2, (zr + zi) * (-_R2))
        return ((zr + zi) * (-_R2), (zr - zi) * _R2)
    c = float(np.cos(2 * np.pi * m / 16))
    s = float(sign * np.sin(2 * np.pi * m / 16))
    return (zr * c - zi * s, zr * s + zi * c)


def _dft16(x, sign):
    t = []
    for a0 in range(4):
        t.append(_dft4([x[4 * a1 + a0] for a1 in range(4)], sign))
    out = [None] * 16
    for k0 in range(4):
        col = [_twiddle(t[a0][k0], a0 * k0, sign) for a0 in range(4)]
        res = _dft4(col, sign)
        for kh in range(4):
            out[k0 + 4 * kh] = res[kh]
    return out


def _dft5_real(x):
    x0, x1, x2, x3, x4 = x
    s14, d14 = x1 + x4, x1 - x4
    s23, d23 = x2 + x3, x2 - x3
    y0 = x0 + s14 + s23
    a1 = x0 + C1 * s14 + C2 * s23
    a2 = x0 + C2 * s14 + C1 * s23
    b1 = S1 * d14 + S2 * d23
    b2 = S2 * d14 - S1 * d23
    return y0, a1, b1, a2, b2


def _idft5_real(g0, p1, q1, p2, q2):
    ea = g0 + C1 * p1 + C2 * p2
    eb = g0 + C2 * p1 + C1 * p2
    oa = S1 * q1 + S2 * q2
    ob = S2 * q1 - S1 * q2
    return [g0 + p1 + p2, ea - oa, eb - ob, eb + ob, ea + oa]


def _kernel(xa_hbm, wr_hbm, wi_hbm, xb_hbm, wqkv_hbm, wo_hbm,
            gg_hbm, gh_hbm, tw_hbm,
            out_hbm,
            xa_v, xb_v, wk_v, wq_v, wv_v, wo_v, wr_v, wi_v, wl_v, gg_v, gh_v, tw_v,
            ys, ts, kp, khat, qt, vt, wqvt, outa, outb, ssc,
            sem_in, sem_wk, sem_xa, sem_xb, sem_w, sem_oa, sem_ob):
    f32, bf16, u32 = jnp.float32, jnp.bfloat16, jnp.uint32
    nt_dims = (((1,), (1,)), ((), ()))

    def dot(a, b):
        return jnp.dot(a, b, preferred_element_type=f32)

    def dot_nt(a, b):
        return jax.lax.dot_general(a, b, nt_dims, preferred_element_type=f32)

    def mult(v, m):
        return v if isinstance(v, int) else pl.multiple_of(v, m)

    def bc(v):
        return pltpu.bitcast(v, bf16)

    def words(v):
        return pltpu.bitcast(v.astype(bf16), u32)

    def cp_in(src, dst, i):
        return pltpu.make_async_copy(src, dst, sem_in.at[i])

    def xb_copy(i):
        r0 = pl.multiple_of(512 * i, 128)
        return pltpu.make_async_copy(xb_hbm.at[0, pl.ds(r0, 512), :],
                                     xb_v.at[pl.ds(r0, 512), :], sem_xb.at[i])

    c_wk = [pltpu.make_async_copy(wqkv_hbm.at[pl.ds(128 * j, 128), pl.ds(D, D)],
                                  wk_v.at[pl.ds(128 * j, 128), :], sem_wk.at[j]) for j in range(5)]
    c_xa = [pltpu.make_async_copy(xa_hbm.at[0, :, pl.ds(128 * c, 128)],
                                  xa_v.at[pl.ds(S * c, S), :], sem_xa.at[c]) for c in range(5)]
    c_gg = cp_in(gg_hbm, gg_v, 0)
    c_gh = cp_in(gh_hbm, gh_v, 1)
    c_tw = cp_in(tw_hbm, tw_v, 2)
    c_wq = cp_in(wqkv_hbm.at[:, pl.ds(0, D)], wq_v, 3)
    c_wv = cp_in(wqkv_hbm.at[:, pl.ds(2 * D, D)], wv_v, 4)
    c_w = []
    for n, (src, dst) in enumerate(((wr_hbm, wr_v), (wi_hbm, wi_v))):
        for k1 in range(16):
            c_w.append(pltpu.make_async_copy(src.at[pl.ds(0, NF - 1), pl.ds(128 * k1, 128)],
                                             dst.at[pl.ds(320 * k1, 320), :],
                                             sem_w.at[16 * n + k1]))
    c_wl = [cp_in(wr_hbm.at[pl.ds(NF - 1, 1), :], wl_v.at[0], 5),
            cp_in(wi_hbm.at[pl.ds(NF - 1, 1), :], wl_v.at[1], 6)]
    c_wo = cp_in(wo_hbm, wo_v, 7)
    for c in c_wk + [xb_copy(0)]:
        c.start()
    stages = [[xb_copy(2), c_gg, c_gh, c_tw], [xb_copy(3)] + c_xa, [c_wq, c_wv], []]

    lane = jax.lax.broadcasted_iota(jnp.int32, (8, 128), 1)
    sub8 = jax.lax.broadcasted_iota(jnp.int32, (8, 128), 0)
    zeros8 = jnp.zeros((8, 128), f32)
    zero_u = jnp.zeros((8, 128), u32)

    for c in c_wk:
        c.wait()
    xb_copy(1).start()
    lane128 = jax.lax.broadcasted_iota(jnp.int32, (128, 128), 1)

    def k_tile(t):
        w0 = mult(t * 64, 64)
        kb = dot(xb_v[pl.ds(2 * w0, 128), :], wk_v[...])
        tiles = [kb[:, 128 * j:128 * (j + 1)] for j in range(5)]
        for tt in range(6):
            off = (120 * tt) % 128
            a = (120 * tt) // 128
            if off == 0:
                v = tiles[a]
            elif a + 1 < 5:
                sh = 128 - off
                v = jnp.where(lane128 < sh, pltpu.roll(tiles[a], sh, 1),
                              pltpu.roll(tiles[a + 1], sh, 1))
            else:
                v = pltpu.roll(tiles[a], 128 - off, 1)
            kp[pl.ds(w0, 64), pl.ds(128 * tt, 128)] = words(v)

    def w_transpose(src, r0, j):
        wqvt[pl.ds(r0, D // 2), pl.ds(128 * j, 128)] = pltpu.bitcast(
            src[pl.ds(128 * j, 128), :].T, u32)

    lo60 = lane < 60

    def khat_tile(t):
        w0 = 64 * t
        h0 = 48 * t
        for u in range(11):
            tt = u // 2
            for r in range(6):
                av = kp[pl.ds(w0 - 128 + 8 * r, 8), pl.ds(128 * tt, 128)]
                bv = kp[pl.ds(w0 + 16 + 8 * r, 8), pl.ds(128 * tt, 128)]
                if u % 2 == 0:
                    keep_a = lo60
                    bs = pltpu.roll(bv, 60, 1)
                else:
                    keep_a = jnp.logical_not(lo60)
                    bs = pltpu.roll(bv, 68, 1)
                khat[pl.ds(h0 + 8 * r, 8), pl.ds(128 * u, 128)] = jnp.where(keep_a, av, bs)

    def k_body(i, carry):
        for n, cs in enumerate(stages):
            @pl.when(i == n)
            def _(cs=cs):
                for c in cs:
                    c.start()
        xb_copy(i).wait()
        for u in range(4):
            k_tile(4 * i + u)
        return carry
    jax.lax.fori_loop(0, 4, k_body, 0)

    for c in c_xa + [c_gg, c_gh, c_tw]:
        c.wait()
    for c in c_w + c_wl + [c_wo]:
        c.start()
    himask = jnp.uint32(0xFFFF0000)

    def dft_mats(a):
        fr, fi = tw_v[pl.ds(0, 128), :], tw_v[pl.ds(128, 128), :]
        tr, ti = tw_v[pl.ds(256 + a, 1), :], tw_v[pl.ds(272 + a, 1), :]
        mr, mi = fr * tr - fi * ti, fr * ti + fi * tr
        return [v.astype(bf16) for v in (mr, mr + mi, mi - mr)]

    xa_w = xa_v.bitcast(u32)
    wr_w, wi_w, outa_w = wr_v.bitcast(u32), wi_v.bitcast(u32), outa.bitcast(u32)
    fw = [dict() for _ in range(16)]

    def fwd_0(a):
        j, p = a // 2, a % 2
        xe, xo = [], []
        for c in range(5):
            e = xa_w[pl.ds(1024 * c + j, 64, stride=8), :]
            o = xa_w[pl.ds(1024 * c + 512 + j, 64, stride=8), :]
            xe.append(pltpu.bitcast((e << 16) if p == 0 else (e & himask), f32))
            xo.append(pltpu.bitcast((o << 16) if p == 0 else (o & himask), f32))
        ye, yo = _dft5_real(xe), _dft5_real(xo)
        fw[a]['y'] = [jnp.concatenate([ye[i], yo[i]], 0).astype(bf16) for i in range(5)]

    def fwd_1(a):
        y = fw[a].pop('y')
        z0 = dot_nt(bc(gh_v[pl.ds(0, 72), :]), y[0])
        z14 = dot_nt(bc(gg_v[0]), jnp.concatenate([y[1], y[2]], axis=1))
        z23 = dot_nt(bc(gg_v[1]), jnp.concatenate([y[3], y[4]], axis=1))
        zr = jnp.concatenate(
            [z0[0:32], z14[0:32], z23[0:32], z23[64:96], z14[64:96],
             z0[32:64], z14[32:64], z23[32:64], z23[96:128], z14[96:128], z0[128:144]], 0)
        zi = jnp.concatenate(
            [z0[64:96], z14[128:160], z23[128:160], z23[192:224], z14[192:224],
             z0[96:128], z14[160:192], z23[160:192], z23[224:256], z14[224:256],
             jnp.zeros((16, 128), f32)], 0)
        fw[a]['z'] = [(zr + zi).astype(bf16), zi.astype(bf16), zr.astype(bf16)]

    def fwd_2(a):
        z = fw[a].pop('z')
        ms = dft_mats(a)
        k1 = dot(z[0], ms[0])
        k2 = dot(z[1], ms[1])
        k3 = dot(z[2], ms[2])
        ys[a, :, pl.ds(0, 128)] = (k1 - k2)[:RP]
        ys[a, :, pl.ds(128, 128)] = (k1 + k3)[:RP]

    row16 = jax.lax.broadcasted_iota(jnp.int32, (16, 128), 0)
    never = tw_v[pl.ds(0, 8), :] > 2.0

    def qv_tile(t, tok=None):
        x = pltpu.bitcast(xb_v[pl.ds(128 * t, 128), :], u32)
        if tok is not None:
            x0 = jnp.where(never, pltpu.bitcast(tok, u32), x[0:8, 0:128])
            x = jnp.concatenate([jnp.concatenate([x0, x[8:, 0:128]], 0), x[:, 128:]], 1)
        qv = dot_nt(bc(wqvt[pl.ds(0, D), :]), bc(x))
        q = qv[:D + 48] * QSCALE
        for h in range(H):
            tt, i = h // 6, h % 6
            j = (i + 3) % 6
            base = 120 * tt
            for part, (pos, shift) in enumerate(((i, 0), (j, 20 * i - 20 * j))):
                for g in range(2):
                    row = 16 * (VLO[pos] + g)
                    lo, hi = 20 * pos - row, 20 * pos + 20 - row
                    src = base + row + shift
                    if src < 0:
                        v = jnp.concatenate([jnp.zeros((-src, 128), f32), q[0:16 + src]], 0)
                    else:
                        v = q[src:src + 16]
                    keep = None
                    if lo > 0:
                        keep = (row16 >= lo) if keep is None else jnp.logical_and(keep, row16 >= lo)
                    if hi < 16:
                        keep = (row16 < hi) if keep is None else jnp.logical_and(keep, row16 < hi)
                    if keep is not None:
                        v = jnp.where(keep, v, 0.0)
                    qt[pl.ds(16 * (H * t + h) + 8 * g, 8), pl.ds(128 * part, 128)] = words(v)
        for j in range(H // 2):
            r = D + 40 * j
            pieces = [qv[r:r + 16], jnp.where(row16 == 4, 1.0, qv[r + 16:r + 32]),
                      jnp.where(row16 == 0, 1.0, qv[r + 16:r + 32])]
            if j < H // 2 - 1:
                pieces.append(qv[r + 32:r + 48])
            else:
                pieces.append(jnp.concatenate([qv[r + 32:r + 40], zeros8], 0))
            for g, v in enumerate(pieces):
                vt[pl.ds(32 * j + 8 * g, 8), pl.ds(128 * t, 128)] = words(v)
        return qv[0:8]

    def spectrum(r0, wr, wi, tok=None):
        x = [(ys[a, pl.ds(r0, 8), pl.ds(0, 128)], ys[a, pl.ds(r0, 8), pl.ds(128, 128)])
             for a in range(16)]
        if tok is not None:
            x[0] = (jnp.where(never, tok, x[0][0]), x[0][1])
        xf = _dft16(x, -1)
        xw = []
        for k1 in range(16):
            xr, xi = xf[k1]
            ar, ai = wr[k1], wi[k1]
            xw.append((xr * ar - xi * ai, xr * ai + xi * ar))
        return _dft16(xw, +1)

    def put_t(w0, halves):
        for a in range(16):
            tr = jnp.concatenate([halves[0][a][0], halves[1][a][0]], 0)
            ti = jnp.concatenate([halves[0][a][1], halves[1][a][1]], 0)
            for c, v in enumerate((tr + ti, tr, ti)):
                ts[pl.ds(168 * a + w0, 8), pl.ds(128 * c, 128)] = words(v)

    def mid_block(i, tok):
        rho = i // 2
        halves = []
        for hh in range(2):
            st = rho // 2 + 80 * (i % 2) + 40 * hh
            ws = []
            for ref in (wr_w, wi_w):
                w = [ref[pl.ds(160 * k1 + st, 8, stride=5), :] for k1 in range(16)]
                ws.append([pltpu.bitcast((v << 16) if rho % 2 == 0 else (v & himask), f32)
                           for v in w])
            halves.append(spectrum(16 * i + 8 * hh, ws[0], ws[1], tok))
        put_t(8 * i, halves)
        return halves[1][15][1]

    def mid_last():
        wr = [jnp.broadcast_to(wl_v[0, :, pl.ds(128 * k1, 128)].astype(f32), (8, 128))
              for k1 in range(16)]
        wi = [jnp.broadcast_to(wl_v[1, :, pl.ds(128 * k1, 128)].astype(f32), (8, 128))
              for k1 in range(16)]
        put_t(160, [spectrum(320, wr, wi), [(zeros8, zeros8)] * 16])

    for step in range(16 + 3):
        if step == 11:
            c_wq.wait()
            c_wv.wait()
        if 11 <= step < 16:
            w_transpose(wq_v, 0, step - 11)
            w_transpose(wv_v, D // 2, step - 11)
        if step < 16:
            fwd_0(step)
        if 2 <= step < 16:
            khat_tile(step)
        if 0 <= step - 1 < 16:
            fwd_1(step - 1)
        if 0 <= step - 3 < 16:
            fwd_2(step - 3)
    for c in c_w + c_wl:
        c.wait()
    done = 0
    mtk = {}
    for t in range(NT):
        tok = qv_tile(t, mtk.get(t - 4))
        upto = ((t + 1) * 21 + NT - 1) // NT
        for i in range(done, upto):
            if i < 20:
                mtk[t] = mid_block(i, tok)
            else:
                mid_last()
        done = upto

    iv = [dict() for _ in range(16)]
    row32 = jax.lax.broadcasted_iota(jnp.int32, (32, 128), 0)

    def inv_1(a):
        ms = dft_mats(a)
        k1 = dot_nt(bc(ts[pl.ds(168 * a, 168), pl.ds(0, 128)]), ms[0])
        k2 = dot_nt(bc(ts[pl.ds(168 * a, 168), pl.ds(128, 128)]), ms[1])
        k3 = dot_nt(bc(ts[pl.ds(168 * a, 168), pl.ds(256, 128)]), ms[2])
        ur, ui = k1 + k3, k1 - k2

        def rows(v, rhos):
            return [v[32 * r:32 * r + 32] for r in rhos]
        ui0 = jnp.where(row32 == 0, jnp.broadcast_to(ur[320:321], (32, 128)), ui[0:32])
        iv[a]['st'] = [
            jnp.concatenate(rows(ur, (0, 5)) + [ui0] + rows(ui, (5,)), 0).astype(bf16),
            jnp.concatenate(rows(ur, (1, 6, 4, 9)) + rows(ui, (1, 6, 4, 9)), 0).astype(bf16),
            jnp.concatenate(rows(ur, (2, 7, 3, 8)) + rows(ui, (2, 7, 3, 8)), 0).astype(bf16)]

    def inv_2(a):
        st0, st14, st23 = iv[a].pop('st')
        g0 = dot(bc(gh_v[pl.ds(72, 64), :]), st0)
        pq1 = dot(bc(gg_v[2]), st14)
        pq2 = dot(bc(gg_v[3]), st23)
        iv[a]['y'] = _idft5_real(g0, pq1[:128], pq1[128:], pq2[:128], pq2[128:])
        if a % 2 == 1:
            y0, y1 = iv[a - 1].pop('y'), iv[a].pop('y')
            for c in range(5):
                lo = pltpu.bitcast(y0[c].astype(bf16).astype(f32), u32)
                hi = pltpu.bitcast(y1[c].astype(bf16).astype(f32), u32)
                outa_w[pl.ds(1024 * c + a // 2, 128, stride=8), :] = ((lo >> 16) | hi).T

    def inv_step(step):
        if step < 16:
            inv_1(step)
        if 0 <= step - 3 < 16:
            inv_2(step - 3)

    c_outa = [pltpu.make_async_copy(outa.at[pl.ds(S * c, S), :],
                                    out_hbm.at[0, :, pl.ds(128 * c, 128)], sem_oa.at[c])
              for c in range(5)]

    c_wo.wait()
    r128 = jax.lax.broadcasted_iota(jnp.int32, (128, 128), 0)
    upper = r128 > lane128
    lane16 = jax.lax.broadcasted_iota(jnp.int32, (16, 128), 1)
    lomask = [jnp.where(lane16 < 32 * (jj + 1), jnp.uint32(0xFFFFFFFF), jnp.uint32(0))
              for jj in range(3)]
    r96 = jax.lax.broadcasted_iota(jnp.int32, (96, 128), 0)
    l96 = jax.lax.broadcasted_iota(jnp.int32, (96, 128), 1)
    hole = jnp.logical_and(l96 >= r96, l96 < r96 + 32)
    left = l96 < 32 * (r96 // 32 + 1)
    TQ = 2
    LA = 2

    def outb_copy(i):
        return pltpu.make_async_copy(outb.at[pl.ds(128 * i, 128), :],
                                     out_hbm.at[0, pl.ds(128 * i, 128), pl.ds(D, D)],
                                     sem_ob.at[i])

    def stage_a(t, h):
        i, j = h % 6, (h % 6 + 3) % 6
        w0 = mult(t * 64, 64)
        q0 = mult((t * H + h) * 16, 16)
        qa = qt[pl.ds(q0, 16), pl.ds(0, 128)]
        qb = qt[pl.ds(q0, 16), pl.ds(128, 128)]
        pa = [zero_u] * 8
        pa[VLO[i]], pa[VLO[i] + 1] = qa[:8], qa[8:]
        qw = bc(jnp.concatenate(pa, 0))
        ktile = pl.ds(128 * (h // 6), 128)
        if isinstance(t, int) and t < 2:
            sa = jnp.where(upper, NEG, dot(bc(kp[pl.ds(64 * t, 64), ktile]), qw))
            if t == 0:
                return dict(sa=sa, m=jnp.max(sa, axis=0, keepdims=True))
            sb = dot(bc(kp[pl.ds(0, 64), ktile]), qw)
            return dict(sa=sa, sb=sb, m=jnp.max(jnp.maximum(sa, sb), axis=0, keepdims=True))
        xa = dot(bc(kp[pl.ds(w0 - 80, 48), ktile]), qw)
        xb = dot(bc(kp[pl.ds(w0 - 32, 48), ktile]), qw)
        hs = []
        for jj in range(3):
            ql, qh = qa & lomask[jj], qb & ~lomask[jj]
            pb = [zero_u] * 8
            pb[VLO[i]], pb[VLO[i] + 1] = ql[:8], ql[8:]
            pb[VLO[j]], pb[VLO[j] + 1] = qh[:8], qh[8:]
            hs.append(dot(bc(khat[pl.ds(mult(t * 48, 16) + 16 * jj, 16),
                                  pl.ds(128 * (h // 3), 128)]), bc(jnp.concatenate(pb, 0))))
        sh = jnp.where(hole, NEG, jnp.concatenate(hs, 0))
        s0 = jnp.where(upper[96:], xa[:32], NEG)
        s2 = jnp.where(upper[:32], NEG, xb[64:])
        sb = jnp.concatenate([xa[32:], xb[:64]], 0)
        m = jnp.maximum(jnp.maximum(jnp.max(sh, axis=0, keepdims=True),
                                    jnp.max(sb, axis=0, keepdims=True)),
                        jnp.max(jnp.maximum(s0, s2), axis=0, keepdims=True))
        return dict(sh=sh, s0=s0, s2=s2, sb=sb, m=m)

    SLOTS = dict(sh=(0, 96), s0=(96, 32), sb=(128, 128), s2=(256, 32), m=(288, 8))

    def park(j, s_):
        for name, (r0, n) in SLOTS.items():
            ssc[j, pl.ds(r0, n), :] = jnp.broadcast_to(s_[name], (n, 128))

    def attn_body(tb, carry):
        n = H * TQ
        st = [dict() for _ in range(n)]
        early = isinstance(tb, int)

        def tq(k):
            return tb * TQ + k // H

        def stage_e(k):
            s_ = st[k]
            m = s_.pop('m')
            if early:
                s_['p2'] = jnp.exp2(s_.pop('sa') - m).astype(bf16)
            else:
                ph = jnp.exp2(s_.pop('sh') - m)
                s_['p0'] = jnp.concatenate(
                    [jnp.where(left, ph, 0.0), jnp.exp2(s_.pop('s0') - m)], 0).astype(bf16)
                s_['p2'] = jnp.concatenate(
                    [jnp.exp2(s_.pop('s2') - m), jnp.where(left, 0.0, ph)], 0).astype(bf16)
            if 'sb' in s_:
                s_['p1'] = jnp.exp2(s_.pop('sb') - m).astype(bf16)

        def stage_v(k):
            h = k % H
            r0 = mult(tq(k) * 128, 128)
            s_ = st[k]
            r = None
            for c, name in ((0, 'p0'), (2, 'p2'), (1, 'p1')):
                if name not in s_:
                    continue
                d = dot(bc(vt[pl.ds(16 * h, 16), pl.ds(r0 - WIN + 128 * c, 128)]), s_.pop(name))
                r = d if r is None else r + d
            s_['r'] = r
            if h == H - 1:
                groups = []
                for kk in range(k - H + 1, k + 1, 2):
                    ra, rb = st[kk].pop('r'), st[kk + 1].pop('r')
                    ia = 1.0 / ra[20:21]
                    ib = 1.0 / rb[0:1]
                    groups += [ra[0:8] * ia, ra[8:16] * ia,
                               jnp.where(sub8 < 4, ra[16:24] * ia, rb[0:8] * ib),
                               rb[8:16] * ib, rb[16:24] * ib]
                o = jnp.concatenate(groups, axis=0).astype(bf16).T
                outb[pl.ds(r0, 128), :] = dot(o, wo_v[...]).astype(bf16)
                outb_copy(tq(k)).start()

        for k in range(LA):
            if early:
                st[k] = stage_a(0, k)
            else:
                st[k] = {name: ssc[k, pl.ds(r0, 1 if name == 'm' else n), :]
                         for name, (r0, n) in SLOTS.items()}
        for step in range(n + 1):
            if step < n:
                k = step + LA
                if k < n:
                    st[k] = stage_a(tq(k), k % H)
                else:
                    park(k - n, stage_a(TQ if early else jnp.minimum(tb * TQ + TQ, NT - 1), k - n))
                stage_e(step)
            if step >= 1:
                stage_v(step - 1)
            if early and step % 2 == 1 and step // 2 < 19:
                inv_step(step // 2)
        return carry
    attn_body(0, 0)
    for c in c_outa:
        c.start()
    jax.lax.fori_loop(1, NT // TQ, attn_body, 0)

    for c in c_outa:
        c.wait()
    for i in range(NT):
        outb_copy(i).wait()


def _call(xa, wr, wi, xb, wqkv, wo):
    bf16, f32, u32 = jnp.bfloat16, jnp.float32, jnp.uint32
    V = pltpu.VMEM
    scratch = [
        V((5 * S, 128), bf16),
        V((S, D), bf16),
        V((D, D), bf16),
        V((D, D), bf16), V((D, D), bf16),
        V((D, D), bf16),
        V((16 * 320, 128), bf16), V((16 * 320, 128), bf16),
        V((2, 1, S), bf16),
        V((4, 128, 256), u32),
        V((136, 128), u32),
        V((2 * 128 + 2 * 16, 128), f32),
        V((16, RP, 256), f32),
        V((16 * RP16 // 2, 3 * 128), u32),
        V((S // 2, 6 * 128), u32),
        V((NT * 48, 11 * 128), u32),
        V((NT * H * 16, 256), u32),
        V((16 * H, S), u32),
        V((D, D), u32),
        V((5 * S, 128), bf16),
        V((S, D), bf16),
        V((2, 296, 128), f32),
        pltpu.SemaphoreType.DMA((8,)),
        pltpu.SemaphoreType.DMA((5,)),
        pltpu.SemaphoreType.DMA((5,)),
        pltpu.SemaphoreType.DMA((4,)),
        pltpu.SemaphoreType.DMA((32,)),
        pltpu.SemaphoreType.DMA((5,)),
        pltpu.SemaphoreType.DMA((NT,)),
    ]
    any_spec = pl.BlockSpec(memory_space=pl.ANY)
    return pl.pallas_call(
        _kernel,
        out_shape=jax.ShapeDtypeStruct((1, S, 2 * D), bf16),
        in_specs=[any_spec] * 9,
        out_specs=any_spec,
        scratch_shapes=scratch,
        compiler_params=pltpu.CompilerParams(vmem_limit_bytes=100 * 1024 * 1024),
    )(xa, wr.T, wi.T, xb, wqkv, wo, _GG, _GH, _TW)


@jax.jit
def pallas_concat_heads__spectral_gfnet__sliding_block__prompt_kernel(
    A_x: jax.Array,
    A_w_r: jax.Array,
    A_w_i: jax.Array,
    B_x: jax.Array,
    B_wqkv: jax.Array,
    B_wo: jax.Array,
):
    return _call(A_x, A_w_r, A_w_i, B_x, B_wqkv, B_wo)
```
